```python
import jax
import jax.numpy as jnp

def _softmax(x, axis=-1):
    return jax.nn.softmax(x, axis=axis)
def _gelu(x):
    return jax.nn.gelu(x, approximate=True)
def _silu(x):
    return jax.nn.silu(x)
def _sigmoid(x):
    return jax.nn.sigmoid(x)
def _layernorm(x, axis=-1, eps=1e-5):
    m = jnp.mean(x, axis=axis, keepdims=True)
    v = jnp.var(x, axis=axis, keepdims=True)
    return (x - m) / jnp.sqrt(v + eps)
def _scatter_add(tgt, idx, src, axis=0):
    return tgt.at[idx].add(src)
def _segment_sum(src, seg, n):
    return jax.ops.segment_sum(src, seg, n)
class _Rng:
    def __init__(self, key):
        self._k = key
    def _next(self):
        self._k, sub = jax.random.split(self._k)
        return sub
    def normal(self, shape):
        return jax.random.normal(self._next(), shape, dtype=jnp.bfloat16)
    def randint(self, lo, hi, shape):
        return jax.random.randint(self._next(), shape, lo, hi, dtype=jnp.int32)
    def uniform(self, shape, lo=0.0, hi=1.0):
        return jax.random.uniform(self._next(), shape, jnp.bfloat16, lo, hi)
    def permutation(self, n):
        return jax.random.permutation(self._next(), n)


kernel_name = 'gated_mix__gqa_block_cached__dense_activation_relu__decode'

def _fwd_setup_inputs():
    _rng = _Rng(jax.random.key(int.from_bytes(__import__("os").urandom(4), "little")))
    _w = (lambda a: (lambda t: t.astype(jnp.bfloat16) if jnp.issubdtype(t.dtype, jnp.floating) else t)(jnp.asarray(a)))
    def _A_setup():
        B, Sq, D = 2, 1, 512
        Hq, Hkv, Sk, Dh = 32, 8, 8192, 128
        assert Hq % Hkv == 0, (Hq, Hkv)
        return {
            "x": _w((lambda *s: _rng.normal(s) * 0.05)(B, Sq, D)),
            "k_cache": _w((lambda *s: _rng.normal(s) * 0.05)(B, Hkv, Sk, Dh)),
            "v_cache": _w((lambda *s: _rng.normal(s) * 0.05)(B, Hkv, Sk, Dh)),
            "wq": _w((lambda *s: _rng.normal(s) * 0.05)(D, Hq * Dh) * (D ** -0.5)),
            "wo": _w((lambda *s: _rng.normal(s) * 0.05)(Hq * Dh, D) * ((Hq * Dh) ** -0.5)),
        }
    _A_in = _A_setup()

    def _B_setup():
        B, S, D, Dff = 2, 1, 512, 1792
        return {
            "x": _w((lambda *s: _rng.normal(s) * 0.05)(B, S, D)),
            "w1": _w((lambda *s: _rng.normal(s) * 0.05)(D, Dff)),
            "w2": _w((lambda *s: _rng.normal(s) * 0.05)(Dff, D)),
        }
    _B_in = _B_setup()

    return {
        "A_x": _A_in["x"],
        "A_k_cache": _A_in["k_cache"],
        "A_v_cache": _A_in["v_cache"],
        "A_wq": _A_in["wq"],
        "A_wo": _A_in["wo"],
        "B_x": _B_in["x"],
        "B_w1": _B_in["w1"],
        "B_w2": _B_in["w2"],
        "gate_w": _w((lambda *s: _rng.normal(s) * 0.05)(512)),
    }

def _fwd_reference(A_x, A_k_cache, A_v_cache, A_wq, A_wo, B_x, B_w1, B_w2, gate_w):
    def _A_ref(x, k_cache, v_cache, wq, wo):
        B, Sq, D = x.shape
        Hq, Dh = 32, 128
        Hkv = k_cache.shape[1]
        rep = Hq // Hkv
        q = (lambda x, *d: x.transpose(*d))((x @ wq).reshape(B, Sq, Hq, Dh), 0, 2, 1, 3)
        k = jnp.repeat(k_cache, rep, axis=1)
        v = jnp.repeat(v_cache, rep, axis=1)
        scores = jnp.einsum("bhqd,bhkd->bhqk", q, k) * (Dh ** -0.5)
        p = _softmax(scores, axis=-1)
        o = jnp.einsum("bhqk,bhkd->bhqd", p, v)
        return (lambda x, *d: x.transpose(*d))(o, 0, 2, 1, 3).reshape(B, Sq, Hq * Dh) @ wo

    def _B_ref(x, w1, w2):
        h = jnp.einsum("bsd,df->bsf", x, w1)
        zero = jnp.zeros_like(h)
        h = jnp.maximum(h, zero)
        return jnp.einsum("bsf,fd->bsd", h, w2)

    x = A_x
    g = _sigmoid((x * gate_w).sum(-1, keepdims=True))
    a = _A_ref(x, A_k_cache, A_v_cache, A_wq, A_wo)
    b = _B_ref(x, B_w1, B_w2)
    return g * a + (1 - g) * b


def setup_inputs():
    _inp = _fwd_setup_inputs()
    _gk = jax.random.fold_in(jax.random.key(int.from_bytes(__import__("os").urandom(4), "little")), 2**31 - 1)
    _shapes = [[2, 1, 512]]
    _dtypes = ['bfloat16']
    _gks = jax.random.split(_gk, len(_shapes))
    _gs = [jax.random.normal(k, s, dtype=jnp.dtype(d)) * 0.05 for k, s, d in zip(_gks, _shapes, _dtypes)]
    _inp["grad_out"] = _gs[0]
    return _inp

def reference(A_x, A_k_cache, A_v_cache, A_wq, A_wo, B_w1, B_w2, gate_w, B_x, grad_out):
    _const = dict(B_x=B_x)
    def _f(*_d):
        return _fwd_reference(**{'A_x': _d[0], 'A_k_cache': _d[1], 'A_v_cache': _d[2], 'A_wq': _d[3], 'A_wo': _d[4], 'B_w1': _d[5], 'B_w2': _d[6], 'gate_w': _d[7], **_const})
    _out, _vjp = jax.vjp(_f, A_x, A_k_cache, A_v_cache, A_wq, A_wo, B_w1, B_w2, gate_w)
    _grads = _vjp(grad_out)
    _out0 = jnp.asarray(_out)
    return (_out0, *[jnp.asarray(_g) for _g in _grads])
```

```python
import contextlib
import jax
import jax.numpy as jnp
from jax import lax
import jax.experimental.pallas as pl
import jax.experimental.pallas.tpu as pltpu

F32, BF16 = jnp.float32, jnp.bfloat16
NN = (((1,), (0,)), ((), ()))
NT = (((1,), (1,)), ((), ()))
TN = (((0,), (0,)), ((), ()))

B, D = 2, 512
HQ, HKV, SK, DH = 32, 8, 8192, 128
REP = HQ // HKV
R8 = B * REP
DFF = 1792
GW = REP * DH
SEG = 4096
NSEG = SK // SEG
FC = 256


def make(piece=64, streams=8, first=60, per_step=6, tail=1024, n_early=4, CH=1024, bounds=False, scopes=False,
         unroll1=8, unroll3=8, unroll4=8):
    scope = jax.named_scope if scopes else (lambda name: contextlib.nullcontext())
    nseg = B * HKV * NSEG
    n_round = SEG // piece
    gph = HKV * NSEG // streams
    n_kv_rounds = 2 * B * gph * n_round
    n_ch = SEG // CH

    def kernel(x_hbm, k_hbm, v_hbm, wq_hbm, wo_hbm, w1_hbm, w2_hbm, gw_hbm, go_hbm,
               out_hbm, dx_hbm, dk_hbm, dv_hbm, dwq_hbm, dwo_hbm, dw1_hbm, dw2_hbm, dgw_hbm,
               kb, vb, wq_v, wo_v, w1_v, w2_v, x_v, go_v, gw_v,
               out_v, dx_v, dgw_v, q_s, do_s, s_s, dp_s, pd_s,
               sem_w, sem_kv, sem_out):

        rd_wq, rd_x, rd_go, rd_gw, rd_wo, rd_w1, rd_w2 = (
            pltpu.make_async_copy(src, dst, sem_w.at[i]) for i, (src, dst) in enumerate((
                (wq_hbm, wq_v), (x_hbm, x_v), (go_hbm, go_v), (gw_hbm, gw_v),
                (wo_hbm, wo_v), (w1_hbm, w1_v), (w2_hbm, w2_v))))

        def rd_kv(h):
            cps = []
            for b in range(B):
                s0 = (b * HKV + h) * NSEG
                seg = pl.ds(s0, NSEG)
                cps.append(pltpu.make_async_copy(k_hbm.at[seg], kb.at[seg], sem_kv.at[h]))
                if b < B - 1:
                    cps.append(pltpu.make_async_copy(v_hbm.at[seg], vb.at[seg], sem_kv.at[h]))
                else:
                    seg, s1 = pl.ds(s0, NSEG - 1), s0 + NSEG - 1
                    r0, r1 = pl.ds(0, SEG - tail), pl.ds(SEG - tail, tail)
                    cps.append(pltpu.make_async_copy(v_hbm.at[seg], vb.at[seg], sem_kv.at[h]))
                    cps.append(pltpu.make_async_copy(v_hbm.at[s1, r0], vb.at[s1, r0], sem_kv.at[h]))
                    cps.append(pltpu.make_async_copy(v_hbm.at[s1, r1], vb.at[s1, r1], sem_kv.at[HKV + h]))
            return cps

        for c in (rd_wq, rd_x, rd_go, rd_gw, rd_wo, rd_w1, rd_w2):
            c.start()

        @pl.loop(0, HKV)
        def _(h):
            for c in rd_kv(h):
                c.start()

        def wr_kv(r):
            grp, c = r // n_round, r % n_round
            seg = pl.ds((((grp // 2) % B) * gph + grp // (2 * B)) * streams, streams)
            rows = pl.ds(pl.multiple_of(c * piece, piece), piece)

            @pl.when(grp % 2 == 0)
            def _():
                pltpu.make_async_copy(kb.at[seg, rows], dk_hbm.at[seg, rows], sem_out.at[0]).start()

            @pl.when(grp % 2 == 1)
            def _():
                pltpu.make_async_copy(vb.at[seg, rows], dv_hbm.at[seg, rows], sem_out.at[0]).start()

        row = lax.broadcasted_iota(jnp.int32, (R8, D), 0)
        row_h = lax.broadcasted_iota(jnp.int32, (R8, DH), 0)

        def rep_rows(a):
            return jnp.where(row < REP, a[0:1], a[1:2])

        def to_heads(full):
            acc = full[:, :DH]
            for j in range(1, REP):
                acc = jnp.where(row_h % REP == j, full[:, j * DH:(j + 1) * DH], acc)
            return acc

        def from_heads(a):
            return jnp.concatenate([jnp.where(row_h % REP == j, a, 0.0) for j in range(REP)], axis=1)

        rd_x.wait()
        rd_go.wait()
        rd_gw.wait()
        x8 = rep_rows(x_v[...].astype(F32))
        go8 = rep_rows(go_v[...].astype(F32))
        gw4 = gw_v[...].astype(F32)
        gw1 = jnp.concatenate([gw4[i:i + 1] for i in range(D // 128)], axis=1)
        g8 = jax.nn.sigmoid(jnp.sum(x8 * gw1, axis=1, keepdims=True))
        x8b = x8.astype(BF16)
        da8b = (g8 * go8).astype(BF16)
        db8b = jnp.where(row % REP == 0, (1.0 - g8) * go8, 0.0).astype(BF16)

        rd_wq.wait()

        @pl.loop(0, HKV)
        def _(h):
            cols = pl.ds(pl.multiple_of(h * GW, GW), GW)
            q_s[h] = to_heads(lax.dot_general(x8b, wq_v[:, cols], NN, preferred_element_type=F32))

        with scope("wait_wo"):
            rd_wo.wait()

        @pl.loop(0, HKV)
        def _(h):
            rows = pl.ds(pl.multiple_of(h * GW, GW), GW)
            do_s[h] = to_heads(lax.dot_general(da8b, wo_v[rows, :], NT, preferred_element_type=F32))

        with scope("wait_w12"):
            rd_w1.wait()
            rd_w2.wait()

        def ffn(i, acc):
            blk = pl.ds(pl.multiple_of(i * FC, FC), FC)
            w1, w2 = w1_v[:, blk], w2_v[blk, :]
            hid = lax.dot_general(x8b, w1, NN, preferred_element_type=F32)
            act = jnp.maximum(hid, 0.0).astype(BF16)
            dact = lax.dot_general(db8b, w2, NT, preferred_element_type=F32)
            slope = jnp.where(hid > 0.0, 1.0, jnp.where(hid == 0.0, 0.5, 0.0))
            dhid = (dact * slope).astype(BF16)
            b8 = acc[0] + lax.dot_general(act, w2, NN, preferred_element_type=F32)
            dx8 = acc[1] + lax.dot_general(dhid, w1, NT, preferred_element_type=F32)
            w2_v[blk, :] = lax.dot_general(act, db8b, TN, preferred_element_type=F32).astype(BF16)
            w1_v[:, blk] = lax.dot_general(x8b, dhid, TN, preferred_element_type=F32).astype(BF16)
            return b8, dx8

        b8, dx8 = lax.fori_loop(0, DFF // FC, ffn, (jnp.zeros((R8, D), F32),) * 2)

        scale = DH ** -0.5

        def chunk(i):
            sg, c = i // n_ch, i % n_ch
            return sg, pl.ds(pl.multiple_of(c * CH, CH), CH), pl.ds(pl.multiple_of(i * CH, CH), CH)

        def softmax_and_projections(h, a8, dx8):
            q, do = q_s[h], do_s[h]
            qb, dob = q.astype(BF16), do.astype(BF16)
            seg0 = [(b * HKV + h) * NSEG for b in range(B)]
            row_c = lax.broadcasted_iota(jnp.int32, (R8, CH), 0)

            @pl.loop(0, NSEG * n_ch, unroll=unroll1)
            def _(i):
                sg, rows, cols = chunk(i)
                s = [lax.dot_general(qb, kb[seg0[b] + sg, rows, :], NT, preferred_element_type=F32)
                     for b in range(B)]
                s_s[:, cols] = jnp.where(row_c < REP, s[0], s[1]) * scale
                dp = [lax.dot_general(dob, vb[seg0[b] + sg, rows, :], NT, preferred_element_type=F32)
                      for b in range(B)]
                dp_s[:, cols] = jnp.where(row_c < REP, dp[0], dp[1])

            s = s_s[...]
            e = jnp.exp(s - jnp.max(s, axis=1, keepdims=True))
            p = e / jnp.sum(e, axis=1, keepdims=True)
            dp = dp_s[...]
            ds = p * (dp - jnp.sum(p * dp, axis=1, keepdims=True)) * scale
            pd_s[h] = jnp.concatenate([p, ds], axis=0).astype(BF16)

            def pv(i, acc):
                sg, rows, cols = chunk(i)
                pd = pd_s[h, :, cols]
                new = []
                for b in range(B):
                    new.append(acc[2 * b] + lax.dot_general(
                        pd, vb[seg0[b] + sg, rows, :], NN, preferred_element_type=F32))
                    new.append(acc[2 * b + 1] + lax.dot_general(
                        pd, kb[seg0[b] + sg, rows, :], NN, preferred_element_type=F32))
                return tuple(new)

            o0, dq0, o1, dq1 = lax.fori_loop(
                0, NSEG * n_ch, pv, (jnp.zeros((2 * R8, DH), F32),) * (2 * B), unroll=unroll3)
            ro = from_heads(jnp.where(row_h < REP, o0[:R8], o1[:R8])).astype(BF16)
            rq = from_heads(jnp.where(row_h < REP, dq0[R8:], dq1[R8:])).astype(BF16)
            blk = pl.ds(pl.multiple_of(h * GW, GW), GW)
            a8 = a8 + lax.dot_general(ro, wo_v[blk, :], NN, preferred_element_type=F32)
            dx8 = dx8 + lax.dot_general(rq, wq_v[:, blk], NT, preferred_element_type=F32)
            wo_v[blk, :] = lax.dot_general(ro, da8b, TN, preferred_element_type=F32).astype(BF16)
            wq_v[:, blk] = lax.dot_general(x8b, rq, TN, preferred_element_type=F32).astype(BF16)
            return a8, dx8

        def cache_grads(h, feed=None):
            q, do = q_s[h], do_s[h]
            seg0 = [(b * HKV + h) * NSEG for b in range(B)]
            zero = jnp.zeros_like(q)
            w = []
            for b in range(B):
                mine = (row_h // REP) == b
                w.append(jnp.concatenate([zero, jnp.where(mine, q, 0.0)], axis=0))
                w.append(jnp.concatenate([jnp.where(mine, do, 0.0), zero], axis=0))
            w = jnp.concatenate(w, axis=1).astype(BF16)

            @pl.loop(0, NSEG * n_ch, unroll=unroll4)
            def _(i):
                if feed is not None:
                    feed(i)
                sg, rows, cols = chunk(i)
                r = lax.dot_general(pd_s[h, :, cols], w, TN, preferred_element_type=F32)
                for b in range(B):
                    kb[seg0[b] + sg, rows, :] = r[:, (2 * b) * DH:(2 * b + 1) * DH].astype(BF16)
                    vb[seg0[b] + sg, rows, :] = r[:, (2 * b + 1) * DH:(2 * b + 2) * DH].astype(BF16)

        def head(h, acc):
            cps = rd_kv(h)
            with scope("wait_kv"):
                for c in cps[:-1]:
                    c.wait()

            @pl.when(h == HKV - 1)
            def _():
                with scope("issue_first"):
                    pl.loop(0, first)(wr_kv)

            cps[-1].wait()
            acc = softmax_and_projections(h, *acc)
            with scope("early_grads"):
                pl.when(h < n_early)(lambda: cache_grads(h))
            return acc

        a8, dx8 = lax.fori_loop(0, HKV, head, (jnp.zeros((R8, D), F32), dx8))

        def per_batch(a):
            return jnp.where(row < REP,
                             jnp.sum(jnp.where(row < REP, a, 0.0), axis=0, keepdims=True),
                             jnp.sum(jnp.where(row < REP, 0.0, a), axis=0, keepdims=True))

        arep = per_batch(a8)
        out8 = g8 * arep + (1.0 - g8) * b8
        dz8 = jnp.sum(go8 * (arep - b8), axis=1, keepdims=True) * g8 * (1.0 - g8)
        dxrep = per_batch(dx8) + dz8 * gw1
        row2 = lax.broadcasted_iota(jnp.int32, (B, D), 0)
        out_v[...] = jnp.where(row2 == 0, out8[0:1], out8[REP:REP + 1]).astype(BF16)
        dx_v[...] = jnp.where(row2 == 0, dxrep[0:1], dxrep[REP:REP + 1]).astype(BF16)
        dgw8 = dz8 * x8
        dgw1 = dgw8[0:1] + dgw8[REP:REP + 1]
        dgw_v[...] = jnp.concatenate(
            [dgw1[:, i * 128:(i + 1) * 128] for i in range(D // 128)], axis=0).astype(BF16)

        small = [pltpu.make_async_copy(out_v, out_hbm, sem_out.at[1]),
                 pltpu.make_async_copy(dx_v, dx_hbm, sem_out.at[1]),
                 pltpu.make_async_copy(dgw_v, dgw_hbm, sem_out.at[1])]
        for c in small:
            c.start()

        ready = n_kv_rounds // gph

        @pl.loop(n_early, HKV)
        def _(h):
            def feed(i):
                lo = first + ((h - n_early) * NSEG * n_ch + i) * per_step
                pl.loop(jnp.minimum(lo, ready), jnp.minimum(lo + per_step, ready))(wr_kv)
            with scope("late_grads"):
                cache_grads(h, feed)

        fed = min(first + (HKV - n_early) * NSEG * n_ch * per_step, ready)
        with scope("issue_rest"):
            pl.loop(fed, n_kv_rounds)(wr_kv)

        with scope("issue_w"):
            @pl.loop(0, 64)
            def _(i):
                for j in range(4):
                    rows = pl.ds(pl.multiple_of(j * 128 + (i // 4) * 8, 8), 8)
                    cols = pl.ds(pl.multiple_of((i % 4) * 1024, 1024), 1024)
                    pltpu.make_async_copy(wq_v.at[rows, cols], dwq_hbm.at[rows, cols], sem_out.at[2]).start()
                for j in range(4):
                    rows = pl.ds(pl.multiple_of(j * 1024 + i * 16, 16), 16)
                    pltpu.make_async_copy(wo_v.at[rows], dwo_hbm.at[rows], sem_out.at[2]).start()
                rows = pl.ds(pl.multiple_of(i * 8, 8), 8)
                pltpu.make_async_copy(w1_v.at[rows], dw1_hbm.at[rows], sem_out.at[2]).start()

                @pl.when(i < 56)
                def _():
                    for j in range(2):
                        rows = pl.ds(pl.multiple_of(j * 896 + i * 16, 16), 16)
                        pltpu.make_async_copy(w2_v.at[rows], dw2_hbm.at[rows], sem_out.at[2]).start()

        with scope("wait_all"):
            for c in small:
                c.wait()
            pltpu.make_async_copy(kb, dk_hbm, sem_out.at[0]).wait()
            pltpu.make_async_copy(vb, dv_hbm, sem_out.at[0]).wait()
            for src, dst in ((wq_v, dwq_hbm), (wo_v, dwo_hbm), (w1_v, dw1_hbm), (w2_v, dw2_hbm)):
                pltpu.make_async_copy(src, dst, sem_out.at[2]).wait()

    sds = lambda *s: jax.ShapeDtypeStruct(s, BF16)
    vm = lambda *s: pltpu.VMEM(s, BF16)
    hbm = pl.BlockSpec(memory_space=pltpu.HBM)
    call = pl.pallas_call(
        kernel,
        out_shape=(sds(B, D), sds(B, D), sds(nseg, SEG, DH), sds(nseg, SEG, DH),
                   sds(D, HQ * DH), sds(HQ * DH, D), sds(D, DFF), sds(DFF, D), sds(D // 128, 128)),
        in_specs=[hbm] * 9,
        out_specs=(hbm,) * 9,
        scratch_shapes=[
            vm(nseg, SEG, DH), vm(nseg, SEG, DH), vm(D, HQ * DH), vm(HQ * DH, D), vm(D, DFF), vm(DFF, D),
            vm(B, D), vm(B, D), vm(D // 128, 128),
            vm(B, D), vm(B, D), vm(D // 128, 128),
            pltpu.VMEM((HKV, R8, DH), F32), pltpu.VMEM((HKV, R8, DH), F32),
            pltpu.VMEM((R8, SK), F32), pltpu.VMEM((R8, SK), F32),
            pltpu.VMEM((HKV, 2 * R8, SK), BF16),
            pltpu.SemaphoreType.DMA((7,)), pltpu.SemaphoreType.DMA((2 * HKV,)), pltpu.SemaphoreType.DMA((3,)),
        ],
        compiler_params=pltpu.CompilerParams(vmem_limit_bytes=110 * 1024 * 1024,
                                             disable_bounds_checks=not bounds),
        name="gated_mix_gqa_relu_decode",
    )

    @jax.jit
    def fn(A_x, A_k_cache, A_v_cache, A_wq, A_wo, B_x, B_w1, B_w2, gate_w, grad_out):
        out, dx, dk, dv, dwq, dwo, dw1, dw2, dgw = call(
            A_x.reshape(B, D), A_k_cache.reshape(nseg, SEG, DH), A_v_cache.reshape(nseg, SEG, DH),
            A_wq, A_wo, B_w1, B_w2, gate_w.reshape(D // 128, 128), grad_out.reshape(B, D))
        return (out.reshape(A_x.shape), dx.reshape(A_x.shape), dk.reshape(A_k_cache.shape),
                dv.reshape(A_v_cache.shape), dwq, dwo, dw1, dw2, dgw.reshape(gate_w.shape))
    return fn


_fn = make()


@jax.jit
def pallas_gated_mix__gqa_block_cached__dense_activation_relu__decode_kernel(
        A_x, A_k_cache, A_v_cache, A_wq, A_wo, B_x, B_w1, B_w2, gate_w, grad_out):
    return _fn(A_x, A_k_cache, A_v_cache, A_wq, A_wo, B_x, B_w1, B_w2, gate_w, grad_out)
```

```python
import contextlib
import jax
import jax.numpy as jnp
from jax import lax
import jax.experimental.pallas as pl
import jax.experimental.pallas.tpu as pltpu

F32, BF16 = jnp.float32, jnp.bfloat16
NN = (((1,), (0,)), ((), ()))
NT = (((1,), (1,)), ((), ()))
TN = (((0,), (0,)), ((), ()))

B, D = 2, 512
HQ, HKV, SK, DH = 32, 8, 8192, 128
REP = HQ // HKV
R8 = B * REP
DFF = 1792
GW = REP * DH
FC = 256
SEG = 4096
NSEG = SK // SEG
RPH = 64
RP = SEG // RPH
LO, HI = 1, 0


def make(CH=1024, bounds=False, scopes=False, lead=24, tail=6, no_compute=False, wpiece=64, WC=512,
         semchk=True, long_runs=False, per_step=32):
    scope = jax.named_scope if scopes else (lambda name: contextlib.nullcontext())

    def dot(a, b, dims):
        return lax.dot_general(a, b, dims, preferred_element_type=F32)

    def ds(i, n):
        return pl.ds(i * n, n) if isinstance(i, int) else pl.ds(pl.multiple_of(i * n, n), n)

    def copy(src, dst, idx, sem):
        return pltpu.make_async_copy(src.at[idx], dst.at[idx], sem)

    def kernel(x_hbm, k_hbm, v_hbm, wq_hbm, wo_hbm, w1_hbm, w2_hbm, gw_hbm, go_hbm,
               out_hbm, dx_hbm, dk_hbm, dv_hbm, dwq_hbm, dwo_hbm, dw1_hbm, dw2_hbm, dgw_hbm,
               kb, vb, wq_v, wo_v, w1_v, w2_v, x_v, go_v, gw_v,
               out_v, dx_v, dgw_v, q_s, do_s, s_s, dp_s, pd_s, sem_out):

        row = lax.broadcasted_iota(jnp.int32, (R8, D), 0)
        row_h = lax.broadcasted_iota(jnp.int32, (R8, DH), 0)

        def read_phase(sem_w, sem_kv):
            def rd_qo(c):
                for half in range(2):
                    part = pl.ds(2 * half, 2)
                    copy(wq_hbm, wq_v, (part, ds(c // 4, 8), ds(c % 4, 1024)), sem_w.at[0]).start(priority=LO)
                    copy(wo_hbm, wo_v, (part, ds(c, 16)), sem_w.at[0]).start(priority=HI)

            def rd_w12(c):
                copy(w1_hbm, w1_v, (c % 4, ds(c // 4, 8)), sem_w.at[1]).start(priority=LO)

                @pl.when(c < 56)
                def _():
                    copy(w2_hbm, w2_v, ((2 * c) % 7, ds(c // 7, 32)), sem_w.at[1]).start(priority=HI)

            def rd_kv_at(h, c):
                last = int(c >= RPH - tail) if isinstance(c, int) else jnp.where(c >= RPH - tail, 1, 0)
                sem = sem_kv.at[2 * h + last]
                for b in range(B):
                    idx = (pl.ds((b * HKV + h) * NSEG, NSEG), ds(c, RP))
                    copy(k_hbm, kb, idx, sem).start(priority=LO)
                    copy(v_hbm, vb, idx, sem).start(priority=HI)

            def rd_kv(r):
                rd_kv_at(r // RPH, r % RPH)

            def wait_kv(h, last):
                rows = tail * RP if last else SEG - tail * RP
                for src, dst in ((k_hbm, kb), (v_hbm, vb)):
                    idx = (pl.ds(0, B * NSEG), pl.ds(0, rows))
                    copy(src, dst, idx, sem_kv.at[2 * h + last]).wait()

            small_in = [pltpu.make_async_copy(x_hbm, x_v, sem_w.at[2]),
                        pltpu.make_async_copy(go_hbm, go_v, sem_w.at[2]),
                        pltpu.make_async_copy(gw_hbm, gw_v, sem_w.at[2])]

            rd_qo(0)
            for c in small_in:
                c.start()
            with scope("A"):
                pl.loop(1, 64)(rd_qo)
                pl.loop(0, 2 * lead)(rd_w12)

            def rep_rows(a):
                return jnp.where(row < REP, a[0:1], a[1:2])

            def to_heads(full):
                acc = full[:, :DH]
                for j in range(1, REP):
                    acc = jnp.where(row_h % REP == j, full[:, j * DH:(j + 1) * DH], acc)
                return acc

            def from_heads(a):
                return jnp.concatenate([jnp.where(row_h % REP == j, a, 0.0) for j in range(REP)], axis=1)

            for c in small_in:
                c.wait()
            x8 = rep_rows(x_v[...].astype(F32))
            go8 = rep_rows(go_v[...].astype(F32))
            gw4 = gw_v[...].astype(F32)
            gw1 = jnp.concatenate([gw4[i:i + 1] for i in range(D // 128)], axis=1)
            g8 = jax.nn.sigmoid(jnp.sum(x8 * gw1, axis=1, keepdims=True))
            x8b = x8.astype(BF16)
            da8b = (g8 * go8).astype(BF16)
            db8b = jnp.where(row % REP == 0, (1.0 - g8) * go8, 0.0).astype(BF16)

            def wo_rows(h):
                return h // 2, ds(h % 2, GW)

            with scope("wait_qo"):
                pltpu.make_async_copy(wq_hbm, wq_v, sem_w.at[0]).wait()
                pltpu.make_async_copy(wo_hbm, wo_v, sem_w.at[0]).wait()
            pl.loop(2 * lead, 64)(rd_w12)

            with scope("B"):
                @pl.loop(0, HKV)
                def _(h):
                    pl.loop(h * (lead // 8), (h + 1) * (lead // 8))(rd_kv)
                    q_s[h] = to_heads(dot(x8b, wq_v[:, :, ds(h, GW)].reshape(D, GW), NN))
                    do_s[h] = to_heads(dot(da8b, wo_v[wo_rows(h)], NT))

            with scope("wait_w12"):
                pltpu.make_async_copy(w1_hbm, w1_v, sem_w.at[1]).wait()
                pltpu.make_async_copy(w2_hbm, w2_v, sem_w.at[1]).wait()

            def ffn(i, acc):
                pl.loop(lead + 8 * i, lead + 8 * i + 8)(rd_kv)
                blk = ds(i, FC)
                w1, w2 = w1_v[:, :, blk].reshape(D, FC), w2_v[i]
                hid = dot(x8b, w1, NN)
                act = jnp.maximum(hid, 0.0).astype(BF16)
                slope = jnp.where(hid > 0.0, 1.0, jnp.where(hid == 0.0, 0.5, 0.0))
                dhid = (dot(db8b, w2, NT) * slope).astype(BF16)
                b8 = acc[0] + dot(act, w2, NN)
                dx8 = acc[1] + dot(dhid, w1, NT)
                w2_v[i] = dot(act, db8b, TN).astype(BF16)
                w1_v[:, :, blk] = dot(x8b, dhid, TN).astype(BF16).reshape(4, D // 4, FC)
                return b8, dx8

            with scope("D"):
                b8, dx8 = lax.fori_loop(0, DFF // FC, ffn, (jnp.zeros((R8, D), F32),) * 2)
                pl.loop(lead + 56, lead + 64)(rd_kv)

            def wr_early():
                @pl.loop(0, 16)
                def _(c):
                    copy(w1_v, dw1_hbm, (slice(None), ds(c, 8)), sem_out).start()
                    copy(wo_v, dwo_hbm, (slice(None), ds(c, 32)), sem_out).start()
                    copy(w2_v, dw2_hbm, (slice(None), ds(c, 16)), sem_out).start()
                    copy(wo_v, dwo_hbm, (pl.ds(0, 3), ds(16 + c, 32)), sem_out).start()

            scale = DH ** -0.5
            n_ch = SEG // CH
            n_all = NSEG * n_ch

            def head(h, acc):
                a8, dx8 = acc
                count = [0]

                def tick(n=1):
                    for _ in range(n):
                        ahead, c = divmod(lead + count[0], RPH)
                        count[0] += 1
                        nxt = h + 1 + ahead
                        pl.when(nxt < HKV)(lambda: rd_kv_at(nxt, c))

                with scope("wait_kv"):
                    wait_kv(h, 0)

                @pl.when(h == HKV - 1)
                def _():
                    with scope("kick"):
                        wr_early()

                with scope("wait_kv_tail"):
                    wait_kv(h, 1)
                qb, dob = q_s[h].astype(BF16), do_s[h].astype(BF16)
                seg0 = [(b * HKV + h) * NSEG for b in range(B)]
                row_c = lax.broadcasted_iota(jnp.int32, (R8, CH), 0)

                if not no_compute:
                    for i in range(n_all):
                        sg, rows, cols = i // n_ch, ds(i % n_ch, CH), ds(i, CH)
                        s = []
                        for b in range(B):
                            tick()
                            s.append(dot(qb, kb[seg0[b] + sg, rows, :], NT))
                        s_s[:, cols] = jnp.where(row_c < REP, s[0], s[1]) * scale
                        dp = []
                        for b in range(B):
                            tick()
                            dp.append(dot(dob, vb[seg0[b] + sg, rows, :], NT))
                        dp_s[:, cols] = jnp.where(row_c < REP, dp[0], dp[1])

                    tick(2)
                    s = s_s[...]
                    e = jnp.exp(s - jnp.max(s, axis=1, keepdims=True))
                    p = e / jnp.sum(e, axis=1, keepdims=True)
                    tick(2)
                    dp = dp_s[...]
                    dsc = p * (dp - jnp.sum(p * dp, axis=1, keepdims=True)) * scale
                    pd_s[h] = jnp.concatenate([p, dsc], axis=0).astype(BF16)

                    o = [jnp.zeros((2 * R8, DH), F32)] * B
                    dq = [jnp.zeros((2 * R8, DH), F32)] * B
                    for i in range(n_all):
                        sg, rows, cols = i // n_ch, ds(i % n_ch, CH), ds(i, CH)
                        for b in range(B):
                            tick()
                            pd = pd_s[h, :, cols]
                            o[b] = o[b] + dot(pd, vb[seg0[b] + sg, rows, :], NN)
                            dq[b] = dq[b] + dot(pd, kb[seg0[b] + sg, rows, :], NN)

                    tick(2)
                    ro = from_heads(jnp.where(row_h < REP, o[0][:R8], o[1][:R8])).astype(BF16)
                    rq = from_heads(jnp.where(row_h < REP, dq[0][R8:], dq[1][R8:])).astype(BF16)
                    blk = ds(h, GW)
                    a8 = a8 + dot(ro, wo_v[wo_rows(h)], NN)
                    tick(2)
                    dx8 = dx8 + dot(rq, wq_v[:, :, blk].reshape(D, GW), NT)
                    tick(4)
                    wo_v[wo_rows(h)] = dot(ro, da8b, TN).astype(BF16)
                    tick(4)
                    wq_v[:, :, blk] = dot(x8b, rq, TN).astype(BF16).reshape(4, D // 4, GW)
                tick(RPH - count[0])
                assert count[0] == RPH
                return a8, dx8

            a8, dx8 = lax.fori_loop(0, HKV, head, (jnp.zeros((R8, D), F32), dx8))

            def per_batch(a):
                return jnp.where(row < REP,
                                 jnp.sum(jnp.where(row < REP, a, 0.0), axis=0, keepdims=True),
                                 jnp.sum(jnp.where(row < REP, 0.0, a), axis=0, keepdims=True))

            arep = per_batch(a8)
            out8 = g8 * arep + (1.0 - g8) * b8
            dz8 = jnp.sum(go8 * (arep - b8), axis=1, keepdims=True) * g8 * (1.0 - g8)
            dxrep = per_batch(dx8) + dz8 * gw1
            row2 = lax.broadcasted_iota(jnp.int32, (B, D), 0)
            out_v[...] = jnp.where(row2 == 0, out8[0:1], out8[REP:REP + 1]).astype(BF16)
            dx_v[...] = jnp.where(row2 == 0, dxrep[0:1], dxrep[REP:REP + 1]).astype(BF16)
            dgw8 = dz8 * x8
            dgw1 = dgw8[0:1] + dgw8[REP:REP + 1]
            dgw_v[...] = jnp.concatenate(
                [dgw1[:, i * 128:(i + 1) * 128] for i in range(D // 128)], axis=0).astype(BF16)

        pl.run_scoped(read_phase, pltpu.SemaphoreType.DMA((3,)), pltpu.SemaphoreType.DMA((2 * HKV,)))

        small = [pltpu.make_async_copy(out_v, out_hbm, sem_out),
                 pltpu.make_async_copy(dx_v, dx_hbm, sem_out),
                 pltpu.make_async_copy(dgw_v, dgw_hbm, sem_out)]
        for c in small:
            c.start()

        hpg = 8 // NSEG
        n_wc = SEG // WC
        n_pc = WC // wpiece

        def wr_kv(grp, u, c):
            src, dst = ((kb, dk_hbm), (vb, dv_hbm))[u // B]
            copy(src, dst, (pl.ds((u % B) * HKV * NSEG + grp * 8, 8), ds(c, wpiece)), sem_out).start()

        @pl.loop(0, HKV // hpg * n_wc)
        def _(t):
            grp, i = t // n_wc, t % n_wc
            with scope("grads"):
                if not no_compute:
                    for hh in range(hpg):
                        h = grp * hpg + hh
                        q, do = q_s[h], do_s[h]
                        zero = jnp.zeros_like(q)
                        w = []
                        for b in range(B):
                            mine = (row_h // REP) == b
                            w.append(jnp.concatenate([zero, jnp.where(mine, q, 0.0)], axis=0))
                            w.append(jnp.concatenate([jnp.where(mine, do, 0.0), zero], axis=0))
                        w = jnp.concatenate(w, axis=1).astype(BF16)
                        for sg in range(NSEG):
                            cols = pl.ds(pl.multiple_of(sg * SEG + i * WC, WC), WC)
                            r = dot(pd_s[h, :, cols], w, TN)
                            for b in range(B):
                                seg = (b * HKV + h) * NSEG + sg
                                kb[seg, ds(i, WC), :] = r[:, (2 * b) * DH:(2 * b + 1) * DH].astype(BF16)
                                vb[seg, ds(i, WC), :] = r[:, (2 * b + 1) * DH:(2 * b + 2) * DH].astype(BF16)

            if not long_runs:
                for u in range(4):
                    pl.loop(0, n_pc)(lambda c: wr_kv(grp, u, i * n_pc + c))
            else:
                @pl.when(t < 4)
                def _():
                    for u in range(4):
                        pl.loop(0, n_pc)(lambda c: wr_kv(0, u, t * n_pc + c))

                for u in range(4):
                    @pl.when((t - 8) // 2 == u)
                    def _():
                        pl.loop(0, 2 * n_pc)(lambda c: wr_kv(0, u, (4 + 2 * (t % 2)) * n_pc + c))

        if long_runs:
            for u in range(4):
                pl.loop(0, SEG // wpiece)(lambda c: wr_kv(1, u, c))

        with scope("issue_w"):
            @pl.loop(0, 64)
            def _(c):
                copy(wq_v, dwq_hbm, (slice(None), ds(c // 4, 8), ds(c % 4, 1024)), sem_out).start()
                copy(wo_v, dwo_hbm, (3, ds(64 + c, 8)), sem_out).start()

        with scope("wait_all"):
            for c in small:
                c.wait()
            for src, dst in ((wq_v, dwq_hbm), (wo_v, dwo_hbm), (w1_v, dw1_hbm), (w2_v, dw2_hbm),
                             (kb, dk_hbm), (vb, dv_hbm)):
                pltpu.make_async_copy(src, dst, sem_out).wait()

    sds = lambda *s: jax.ShapeDtypeStruct(s, BF16)
    vm = lambda *s: pltpu.VMEM(s, BF16)
    hbm = pl.BlockSpec(memory_space=pltpu.HBM)
    KV, WQ, WO = (B * HKV * NSEG, SEG, DH), (4, D // 4, HQ * DH), (4, HQ * DH // 4, D)
    W1, W2 = (4, D // 4, DFF), (DFF // FC, FC, D)
    call = pl.pallas_call(
        kernel,
        out_shape=(sds(B, D), sds(B, D), sds(*KV), sds(*KV),
                   sds(*WQ), sds(*WO), sds(*W1), sds(*W2), sds(D // 128, 128)),
        in_specs=[hbm] * 9,
        out_specs=(hbm,) * 9,
        scratch_shapes=[
            vm(*KV), vm(*KV), vm(*WQ), vm(*WO), vm(*W1), vm(*W2),
            vm(B, D), vm(B, D), vm(D // 128, 128),
            vm(B, D), vm(B, D), vm(D // 128, 128),
            pltpu.VMEM((HKV, R8, DH), F32), pltpu.VMEM((HKV, R8, DH), F32),
            pltpu.VMEM((R8, SK), F32), pltpu.VMEM((R8, SK), F32),
            pltpu.VMEM((HKV, 2 * R8, SK), BF16),
            pltpu.SemaphoreType.DMA(()),
        ],
        compiler_params=pltpu.CompilerParams(vmem_limit_bytes=110 * 1024 * 1024,
                                             disable_bounds_checks=not bounds,
                                             disable_semaphore_checks=not semchk),
        name="gated_mix_gqa_relu_decode",
    )

    @jax.jit
    def fn(A_x, A_k_cache, A_v_cache, A_wq, A_wo, B_x, B_w1, B_w2, gate_w, grad_out):
        out, dx, dk, dv, dwq, dwo, dw1, dw2, dgw = call(
            A_x.reshape(B, D), A_k_cache.reshape(KV), A_v_cache.reshape(KV),
            A_wq.reshape(WQ), A_wo.reshape(WO), B_w1.reshape(W1), B_w2.reshape(W2),
            gate_w.reshape(D // 128, 128), grad_out.reshape(B, D))
        return (out.reshape(A_x.shape), dx.reshape(A_x.shape), dk.reshape(A_k_cache.shape),
                dv.reshape(A_v_cache.shape), dwq.reshape(A_wq.shape), dwo.reshape(A_wo.shape),
                dw1.reshape(B_w1.shape), dw2.reshape(B_w2.shape), dgw.reshape(gate_w.shape))
    return fn


_fn = make()


@jax.jit
def pallas_gated_mix__gqa_block_cached__dense_activation_relu__decode_kernel(
        A_x, A_k_cache, A_v_cache, A_wq, A_wo, B_x, B_w1, B_w2, gate_w, grad_out):
    return _fn(A_x, A_k_cache, A_v_cache, A_wq, A_wo, B_x, B_w1, B_w2, gate_w, grad_out)
```

```python
import jax
import jax.numpy as jnp
from jax import lax
import jax.experimental.pallas as pl
import jax.experimental.pallas.tpu as pltpu

F32, BF16 = jnp.float32, jnp.bfloat16
NN = (((1,), (0,)), ((), ()))
NT = (((1,), (1,)), ((), ()))
TN = (((0,), (0,)), ((), ()))

B, D, DFF = 2, 512, 1792
HQ, HKV, SK, DH = 32, 8, 8192, 128
REP = HQ // HKV
ROWS = B * REP
GW = REP * DH
LANES = 128

SEG = 4096
NSEG = SK // SEG
PIECE = 64
ROUNDS = SEG // PIECE
LEAD = 24
TAIL = 6
LO, HI = 1, 0

CHUNK = 1024
FC = 256
GROUP = 8
WC = 512

KV_VIEW = (B * HKV * NSEG, SEG, DH)
WQ_VIEW = (4, D // 4, HQ * DH)
WO_VIEW = (4, HQ * DH // 4, D)
W1_VIEW = (4, D // 4, DFF)
W2_VIEW = (DFF // FC, FC, D)
GATE_VIEW = (D // LANES, LANES)


def _dot(a, b, dims):
    return lax.dot_general(a, b, dims, preferred_element_type=F32)


def _ds(i, n):
    return pl.ds(i * n, n) if isinstance(i, int) else pl.ds(pl.multiple_of(i * n, n), n)


def _copy(src, dst, idx, sem):
    return pltpu.make_async_copy(src.at[idx], dst.at[idx], sem)


def _kernel(x_hbm, k_hbm, v_hbm, wq_hbm, wo_hbm, w1_hbm, w2_hbm, gw_hbm, go_hbm,
            out_hbm, dx_hbm, dk_hbm, dv_hbm, dwq_hbm, dwo_hbm, dw1_hbm, dw2_hbm, dgw_hbm,
            k_v, v_v, wq_v, wo_v, w1_v, w2_v, x_v, go_v, gw_v, out_v, dx_v, dgw_v,
            q_s, do_s, s_s, dp_s, pd_s, sem_out):
    row = lax.broadcasted_iota(jnp.int32, (ROWS, D), 0)
    row_h = lax.broadcasted_iota(jnp.int32, (ROWS, DH), 0)

    def rep_rows(a):
        return jnp.where(row < REP, a[0:1], a[1:2])

    def per_batch(a):
        return jnp.where(row < REP,
                         jnp.sum(jnp.where(row < REP, a, 0.0), axis=0, keepdims=True),
                         jnp.sum(jnp.where(row < REP, 0.0, a), axis=0, keepdims=True))

    def to_heads(full):
        acc = full[:, :DH]
        for j in range(1, REP):
            acc = jnp.where(row_h % REP == j, full[:, j * DH:(j + 1) * DH], acc)
        return acc

    def from_heads(a):
        return jnp.concatenate([jnp.where(row_h % REP == j, a, 0.0) for j in range(REP)], axis=1)

    def wq_cols(h):
        return slice(None), slice(None), _ds(h, GW)

    def wo_rows(h):
        return h // 2, _ds(h % 2, GW)

    def segments(b, h):
        return pl.ds((b * HKV + h) * NSEG, NSEG)

    def read_phase(sem_w, sem_kv):
        def read_qo(c):
            for half in range(2):
                part = pl.ds(2 * half, 2)
                _copy(wq_hbm, wq_v, (part, _ds(c // 4, 8), _ds(c % 4, 1024)), sem_w.at[0]).start(priority=LO)
                _copy(wo_hbm, wo_v, (part, _ds(c, 16)), sem_w.at[0]).start(priority=HI)

        def read_ffn(c):
            _copy(w1_hbm, w1_v, (c % 4, _ds(c // 4, 8)), sem_w.at[1]).start(priority=LO)

            @pl.when(c < 56)
            def _():
                _copy(w2_hbm, w2_v, ((2 * c) % 7, _ds(c // 7, 32)), sem_w.at[1]).start(priority=HI)

        def read_kv(h, c):
            late = c >= ROUNDS - TAIL
            sem = sem_kv.at[2 * h + (int(late) if isinstance(c, int) else late.astype(jnp.int32))]
            for b in range(B):
                idx = (segments(b, h), _ds(c, PIECE))
                _copy(k_hbm, k_v, idx, sem).start(priority=LO)
                _copy(v_hbm, v_v, idx, sem).start(priority=HI)

        def read_kv_rounds(lo, hi):
            pl.loop(lo, hi)(lambda r: read_kv(r // ROUNDS, r % ROUNDS))

        def wait_kv(h, late):
            cut = SEG - TAIL * PIECE
            rows = pl.ds(cut, SEG - cut) if late else pl.ds(0, cut)
            for b in range(B):
                _copy(k_hbm, k_v, (segments(b, h), rows), sem_kv.at[2 * h + late]).wait()
                _copy(v_hbm, v_v, (segments(b, h), rows), sem_kv.at[2 * h + late]).wait()

        small_in = [pltpu.make_async_copy(src, dst, sem_w.at[2])
                    for src, dst in ((x_hbm, x_v), (go_hbm, go_v), (gw_hbm, gw_v))]
        read_qo(0)
        for cp in small_in:
            cp.start()
        pl.loop(1, 64)(read_qo)
        pl.loop(0, 2 * LEAD)(read_ffn)

        for cp in small_in:
            cp.wait()
        x8 = rep_rows(x_v[...].astype(F32))
        go8 = rep_rows(go_v[...].astype(F32))
        gw4 = gw_v[...].astype(F32)
        gw = jnp.concatenate([gw4[i:i + 1] for i in range(D // LANES)], axis=1)
        g = jax.nn.sigmoid(jnp.sum(x8 * gw, axis=1, keepdims=True))
        xb = x8.astype(BF16)
        da = (g * go8).astype(BF16)
        db = jnp.where(row % REP == 0, (1.0 - g) * go8, 0.0).astype(BF16)

        pltpu.make_async_copy(wq_hbm, wq_v, sem_w.at[0]).wait()
        pltpu.make_async_copy(wo_hbm, wo_v, sem_w.at[0]).wait()
        pl.loop(2 * LEAD, 64)(read_ffn)

        @pl.loop(0, HKV)
        def _(h):
            read_kv_rounds(h * (LEAD // HKV), (h + 1) * (LEAD // HKV))
            q_s[h] = to_heads(_dot(xb, wq_v[wq_cols(h)].reshape(D, GW), NN))
            do_s[h] = to_heads(_dot(da, wo_v[wo_rows(h)], NT))

        pltpu.make_async_copy(w1_hbm, w1_v, sem_w.at[1]).wait()
        pltpu.make_async_copy(w2_hbm, w2_v, sem_w.at[1]).wait()

        def ffn(i, acc):
            read_kv_rounds(LEAD + 8 * i, LEAD + 8 * i + 8)
            units = _ds(i, FC)
            w1, w2 = w1_v[:, :, units].reshape(D, FC), w2_v[i]
            hid = _dot(xb, w1, NN)
            act = jnp.maximum(hid, 0.0).astype(BF16)
            slope = jnp.where(hid > 0.0, 1.0, jnp.where(hid == 0.0, 0.5, 0.0))
            dhid = (_dot(db, w2, NT) * slope).astype(BF16)
            ffn_out = acc[0] + _dot(act, w2, NN)
            dx = acc[1] + _dot(dhid, w1, NT)
            w2_v[i] = _dot(act, db, TN).astype(BF16)
            w1_v[:, :, units] = _dot(xb, dhid, TN).astype(BF16).reshape(4, D // 4, FC)
            return ffn_out, dx

        ffn_out, dx = lax.fori_loop(0, DFF // FC, ffn, (jnp.zeros((ROWS, D), F32),) * 2)
        read_kv_rounds(LEAD + 8 * (DFF // FC), LEAD + ROUNDS)

        scale = DH ** -0.5
        n_chunks = SK // CHUNK

        def head(h, acc):
            attn_out, dx = acc
            issued = [0]

            def tick(n=1):
                for _ in range(n):
                    ahead, c = divmod(LEAD + issued[0], ROUNDS)
                    issued[0] += 1
                    nxt = h + 1 + ahead
                    pl.when(nxt < HKV)(lambda: read_kv(nxt, c))

            def cache(ref, b, i):
                return ref[(b * HKV + h) * NSEG + i // (SEG // CHUNK), _ds(i % (SEG // CHUNK), CHUNK), :]

            wait_kv(h, 0)

            @pl.when(h == HKV - 1)
            def _():
                @pl.loop(0, 16)
                def _(c):
                    _copy(w1_v, dw1_hbm, (slice(None), _ds(c, 8)), sem_out).start()
                    _copy(wo_v, dwo_hbm, (slice(None), _ds(c, 32)), sem_out).start()
                    _copy(w2_v, dw2_hbm, (slice(None), _ds(c, 16)), sem_out).start()
                    _copy(wo_v, dwo_hbm, (pl.ds(0, 3), _ds(16 + c, 32)), sem_out).start()

            wait_kv(h, 1)

            q, do = q_s[h].astype(BF16), do_s[h].astype(BF16)
            first = lax.broadcasted_iota(jnp.int32, (ROWS, CHUNK), 0) < REP
            for i in range(n_chunks):
                s, dp = [], []
                for b in range(B):
                    tick()
                    s.append(_dot(q, cache(k_v, b, i), NT))
                s_s[:, _ds(i, CHUNK)] = jnp.where(first, s[0], s[1]) * scale
                for b in range(B):
                    tick()
                    dp.append(_dot(do, cache(v_v, b, i), NT))
                dp_s[:, _ds(i, CHUNK)] = jnp.where(first, dp[0], dp[1])

            tick(2)
            s = s_s[...]
            e = jnp.exp(s - jnp.max(s, axis=1, keepdims=True))
            p = e / jnp.sum(e, axis=1, keepdims=True)
            tick(2)
            dp = dp_s[...]
            dscore = p * (dp - jnp.sum(p * dp, axis=1, keepdims=True)) * scale
            pd_s[h] = jnp.concatenate([p, dscore], axis=0).astype(BF16)

            o = [jnp.zeros((2 * ROWS, DH), F32)] * B
            dq = [jnp.zeros((2 * ROWS, DH), F32)] * B
            for i in range(n_chunks):
                for b in range(B):
                    tick()
                    pd = pd_s[h, :, _ds(i, CHUNK)]
                    o[b] = o[b] + _dot(pd, cache(v_v, b, i), NN)
                    dq[b] = dq[b] + _dot(pd, cache(k_v, b, i), NN)

            tick(2)
            o = from_heads(jnp.where(row_h < REP, o[0][:ROWS], o[1][:ROWS])).astype(BF16)
            dq = from_heads(jnp.where(row_h < REP, dq[0][ROWS:], dq[1][ROWS:])).astype(BF16)
            attn_out = attn_out + _dot(o, wo_v[wo_rows(h)], NN)
            tick(2)
            dx = dx + _dot(dq, wq_v[wq_cols(h)].reshape(D, GW), NT)
            tick(4)
            wo_v[wo_rows(h)] = _dot(o, da, TN).astype(BF16)
            tick(4)
            wq_v[wq_cols(h)] = _dot(xb, dq, TN).astype(BF16).reshape(4, D // 4, GW)
            assert issued[0] == ROUNDS
            return attn_out, dx

        attn_out, dx = lax.fori_loop(0, HKV, head, (jnp.zeros((ROWS, D), F32), dx))

        attn_out = per_batch(attn_out)
        out = g * attn_out + (1.0 - g) * ffn_out
        dz = jnp.sum(go8 * (attn_out - ffn_out), axis=1, keepdims=True) * g * (1.0 - g)
        dx = per_batch(dx) + dz * gw
        batch0 = lax.broadcasted_iota(jnp.int32, (B, D), 0) == 0
        out_v[...] = jnp.where(batch0, out[0:1], out[REP:REP + 1]).astype(BF16)
        dx_v[...] = jnp.where(batch0, dx[0:1], dx[REP:REP + 1]).astype(BF16)
        dgw = dz * x8
        dgw = dgw[0:1] + dgw[REP:REP + 1]
        dgw_v[...] = jnp.concatenate(
            [dgw[:, i * LANES:(i + 1) * LANES] for i in range(D // LANES)], axis=0).astype(BF16)

    pl.run_scoped(read_phase, pltpu.SemaphoreType.DMA((3,)), pltpu.SemaphoreType.DMA((2 * HKV,)))

    small_out = [pltpu.make_async_copy(src, dst, sem_out)
                 for src, dst in ((out_v, out_hbm), (dx_v, dx_hbm), (dgw_v, dgw_hbm))]
    for cp in small_out:
        cp.start()

    heads_per_group = GROUP // NSEG
    steps = SEG // WC

    @pl.loop(0, HKV // heads_per_group * steps)
    def _(t):
        grp, i = t // steps, t % steps
        for j in range(heads_per_group):
            h = grp * heads_per_group + j
            q, do = q_s[h], do_s[h]
            zero = jnp.zeros_like(q)
            w = []
            for b in range(B):
                mine = row_h // REP == b
                w.append(jnp.concatenate([zero, jnp.where(mine, q, 0.0)], axis=0))
                w.append(jnp.concatenate([jnp.where(mine, do, 0.0), zero], axis=0))
            w = jnp.concatenate(w, axis=1).astype(BF16)
            for sg in range(NSEG):
                grads = _dot(pd_s[h, :, _ds(sg * steps + i, WC)], w, TN).astype(BF16)
                for b in range(B):
                    seg = (b * HKV + h) * NSEG + sg
                    k_v[seg, _ds(i, WC), :] = grads[:, 2 * b * DH:(2 * b + 1) * DH]
                    v_v[seg, _ds(i, WC), :] = grads[:, (2 * b + 1) * DH:(2 * b + 2) * DH]

        @pl.when((t == 0) | (t % 2 == 1))
        def _():
            lo = jnp.where(t < 2, i, i - 1)
            for src, dst in ((k_v, dk_hbm), (v_v, dv_hbm)):
                for b in range(B):
                    @pl.loop(lo * (WC // PIECE), (i + 1) * (WC // PIECE))
                    def _(c):
                        part = pl.ds(b * HKV * NSEG + grp * GROUP, GROUP)
                        _copy(src, dst, (part, _ds(c, PIECE)), sem_out).start()

    @pl.loop(0, 64)
    def _(c):
        _copy(wq_v, dwq_hbm, (slice(None), _ds(c // 4, 8), _ds(c % 4, 1024)), sem_out).start()
        _copy(wo_v, dwo_hbm, (3, _ds(64 + c, 8)), sem_out).start()

    for cp in small_out:
        cp.wait()
    for src, dst in ((wq_v, dwq_hbm), (wo_v, dwo_hbm), (w1_v, dw1_hbm), (w2_v, dw2_hbm),
                     (k_v, dk_hbm), (v_v, dv_hbm)):
        pltpu.make_async_copy(src, dst, sem_out).wait()


@jax.jit
def pallas_gated_mix__gqa_block_cached__dense_activation_relu__decode_kernel(
    A_x: jax.Array,
    A_k_cache: jax.Array,
    A_v_cache: jax.Array,
    A_wq: jax.Array,
    A_wo: jax.Array,
    B_x: jax.Array,
    B_w1: jax.Array,
    B_w2: jax.Array,
    gate_w: jax.Array,
    grad_out: jax.Array,
):
    del B_x
    views = (KV_VIEW, KV_VIEW, WQ_VIEW, WO_VIEW, W1_VIEW, W2_VIEW)
    in_hbm = pl.BlockSpec(memory_space=pltpu.HBM)
    out, dx, dk, dv, dwq, dwo, dw1, dw2, dgw = pl.pallas_call(
        _kernel,
        out_shape=tuple(jax.ShapeDtypeStruct(s, BF16) for s in ((B, D), (B, D), *views, GATE_VIEW)),
        in_specs=[in_hbm] * 9,
        out_specs=(in_hbm,) * 9,
        scratch_shapes=[
            *(pltpu.VMEM(s, BF16) for s in (*views, (B, D), (B, D), GATE_VIEW, (B, D), (B, D), GATE_VIEW)),
            pltpu.VMEM((HKV, ROWS, DH), F32),
            pltpu.VMEM((HKV, ROWS, DH), F32),
            pltpu.VMEM((ROWS, SK), F32),
            pltpu.VMEM((ROWS, SK), F32),
            pltpu.VMEM((HKV, 2 * ROWS, SK), BF16),
            pltpu.SemaphoreType.DMA(()),
        ],
        compiler_params=pltpu.CompilerParams(
            vmem_limit_bytes=110 * 1024 * 1024, disable_bounds_checks=True),
        name="gated_mix_gqa_relu_decode",
    )(A_x.reshape(B, D), A_k_cache.reshape(KV_VIEW), A_v_cache.reshape(KV_VIEW),
      A_wq.reshape(WQ_VIEW), A_wo.reshape(WO_VIEW), B_w1.reshape(W1_VIEW), B_w2.reshape(W2_VIEW),
      gate_w.reshape(GATE_VIEW), grad_out.reshape(B, D))
    return (out.reshape(A_x.shape), dx.reshape(A_x.shape),
            dk.reshape(A_k_cache.shape), dv.reshape(A_v_cache.shape),
            dwq.reshape(A_wq.shape), dwo.reshape(A_wo.shape),
            dw1.reshape(B_w1.shape), dw2.reshape(B_w2.shape), dgw.reshape(gate_w.shape))
```

```python
import jax
import jax.numpy as jnp
from jax import lax
import jax.experimental.pallas as pl
import jax.experimental.pallas.tpu as pltpu

F32, BF16 = jnp.float32, jnp.bfloat16
NN = (((1,), (0,)), ((), ()))
NT = (((1,), (1,)), ((), ()))
TN = (((0,), (0,)), ((), ()))

B, D, DFF = 2, 512, 1792
HQ, HKV, SK, DH = 32, 8, 8192, 128
REP = HQ // HKV
ROWS = B * REP
GW = REP * DH
LANES = 128

SEG = 4096
NSEG = SK // SEG
PIECE = 64
ROUNDS = SEG // PIECE
LEAD = 24
TAIL = 6
LO, HI = 1, 0

CHUNK = 1024
FC = 256
GROUP = 8
WC = 512

KV_VIEW = (B * HKV * NSEG, SEG, DH)
WQ_VIEW = (4, D // 4, HQ * DH)
WO_VIEW = (4, HQ * DH // 4, D)
W1_VIEW = (4, D // 4, DFF)
W2_VIEW = (DFF // FC, FC, D)
GATE_VIEW = (D // LANES, LANES)


def _dot(a, b, dims):
    return lax.dot_general(a, b, dims, preferred_element_type=F32)


def _ds(i, n):
    return pl.ds(i * n, n) if isinstance(i, int) else pl.ds(pl.multiple_of(i * n, n), n)


def _copy(src, dst, idx, sem):
    return pltpu.make_async_copy(src.at[idx], dst.at[idx], sem)


def _kernel(x_hbm, k_hbm, v_hbm, wq_hbm, wo_hbm, w1_hbm, w2_hbm, gw_hbm, go_hbm,
            out_hbm, dx_hbm, dk_hbm, dv_hbm, dwq_hbm, dwo_hbm, dw1_hbm, dw2_hbm, dgw_hbm,
            k_v, v_v, wq_v, wo_v, w1_v, w2_v, x_v, go_v, gw_v, out_v, dx_v, dgw_v,
            q_s, do_s, s_s, dp_s, pd_s, sem_out):
    row = lax.broadcasted_iota(jnp.int32, (ROWS, D), 0)
    row_h = lax.broadcasted_iota(jnp.int32, (ROWS, DH), 0)

    def rep_rows(a):
        return jnp.where(row < REP, a[0:1], a[1:2])

    def per_batch(a):
        return jnp.where(row < REP,
                         jnp.sum(jnp.where(row < REP, a, 0.0), axis=0, keepdims=True),
                         jnp.sum(jnp.where(row < REP, 0.0, a), axis=0, keepdims=True))

    def to_heads(full):
        acc = full[:, :DH]
        for j in range(1, REP):
            acc = jnp.where(row_h % REP == j, full[:, j * DH:(j + 1) * DH], acc)
        return acc

    def from_heads(a):
        return jnp.concatenate([jnp.where(row_h % REP == j, a, 0.0) for j in range(REP)], axis=1)

    def wq_cols(h):
        return slice(None), slice(None), _ds(h, GW)

    def wo_rows(h):
        return h // 2, _ds(h % 2, GW)

    def segments(b, h):
        return pl.ds((b * HKV + h) * NSEG, NSEG)

    def read_phase(sem_w, sem_kv):
        def read_qo(c):
            for half in range(2):
                part = pl.ds(2 * half, 2)
                _copy(wq_hbm, wq_v, (part, _ds(c // 4, 8), _ds(c % 4, 1024)), sem_w.at[0]).start(priority=LO)
                _copy(wo_hbm, wo_v, (part, _ds(c, 16)), sem_w.at[0]).start(priority=HI)

        def read_ffn(c):
            _copy(w1_hbm, w1_v, (c % 4, _ds(c // 4, 8)), sem_w.at[1]).start(priority=LO)

            @pl.when(c < 56)
            def _():
                _copy(w2_hbm, w2_v, ((2 * c) % 7, _ds(c // 7, 32)), sem_w.at[1]).start(priority=HI)

        def read_kv(h, c):
            late = c >= ROUNDS - TAIL
            sem = sem_kv.at[2 * h + (int(late) if isinstance(c, int) else late.astype(jnp.int32))]
            for b in range(B):
                idx = (segments(b, h), _ds(c, PIECE))
                _copy(k_hbm, k_v, idx, sem).start(priority=LO)
                _copy(v_hbm, v_v, idx, sem).start(priority=HI)

        def read_kv_rounds(lo, hi):
            pl.loop(lo, hi)(lambda r: read_kv(r // ROUNDS, r % ROUNDS))

        def wait_kv(h, late):
            cut = SEG - TAIL * PIECE
            rows = pl.ds(cut, SEG - cut) if late else pl.ds(0, cut)
            for b in range(B):
                _copy(k_hbm, k_v, (segments(b, h), rows), sem_kv.at[2 * h + late]).wait()
                _copy(v_hbm, v_v, (segments(b, h), rows), sem_kv.at[2 * h + late]).wait()

        small_in = [pltpu.make_async_copy(src, dst, sem_w.at[2])
                    for src, dst in ((x_hbm, x_v), (go_hbm, go_v), (gw_hbm, gw_v))]
        read_qo(0)
        for cp in small_in:
            cp.start()
        pl.loop(1, 64)(read_qo)
        pl.loop(0, 2 * LEAD)(read_ffn)

        for cp in small_in:
            cp.wait()
        x8 = rep_rows(x_v[...].astype(F32))
        go8 = rep_rows(go_v[...].astype(F32))
        gw4 = gw_v[...].astype(F32)
        gw = jnp.concatenate([gw4[i:i + 1] for i in range(D // LANES)], axis=1)
        g = jax.nn.sigmoid(jnp.sum(x8 * gw, axis=1, keepdims=True))
        xb = x8.astype(BF16)
        da = (g * go8).astype(BF16)
        db = jnp.where(row % REP == 0, (1.0 - g) * go8, 0.0).astype(BF16)

        pltpu.make_async_copy(wq_hbm, wq_v, sem_w.at[0]).wait()
        pltpu.make_async_copy(wo_hbm, wo_v, sem_w.at[0]).wait()
        pl.loop(2 * LEAD, 64)(read_ffn)

        @pl.loop(0, HKV)
        def _(h):
            read_kv_rounds(h * (LEAD // HKV), (h + 1) * (LEAD // HKV))
            q_s[h] = to_heads(_dot(xb, wq_v[wq_cols(h)].reshape(D, GW), NN))
            do_s[h] = to_heads(_dot(da, wo_v[wo_rows(h)], NT))

        pltpu.make_async_copy(w1_hbm, w1_v, sem_w.at[1]).wait()
        pltpu.make_async_copy(w2_hbm, w2_v, sem_w.at[1]).wait()

        def ffn(i, acc):
            read_kv_rounds(LEAD + 8 * i, LEAD + 8 * i + 8)
            units = _ds(i, FC)
            w1, w2 = w1_v[:, :, units].reshape(D, FC), w2_v[i]
            hid = _dot(xb, w1, NN)
            act = jnp.maximum(hid, 0.0).astype(BF16)
            slope = jnp.where(hid > 0.0, 1.0, jnp.where(hid == 0.0, 0.5, 0.0))
            dhid = (_dot(db, w2, NT) * slope).astype(BF16)
            ffn_out = acc[0] + _dot(act, w2, NN)
            dx = acc[1] + _dot(dhid, w1, NT)
            w2_v[i] = _dot(act, db, TN).astype(BF16)
            w1_v[:, :, units] = _dot(xb, dhid, TN).astype(BF16).reshape(4, D // 4, FC)
            return ffn_out, dx

        ffn_out, dx = lax.fori_loop(0, DFF // FC, ffn, (jnp.zeros((ROWS, D), F32),) * 2)
        read_kv_rounds(LEAD + 8 * (DFF // FC), LEAD + ROUNDS)

        scale = DH ** -0.5
        n_chunks = SK // CHUNK

        def head(h, acc):
            attn_out, dx = acc
            issued = [0]

            def tick(n=1):
                for _ in range(n):
                    ahead, c = divmod(LEAD + issued[0], ROUNDS)
                    issued[0] += 1
                    nxt = h + 1 + ahead
                    pl.when(nxt < HKV)(lambda: read_kv(nxt, c))

            def cache(ref, b, i):
                return ref[(b * HKV + h) * NSEG + i // (SEG // CHUNK), _ds(i % (SEG // CHUNK), CHUNK), :]

            wait_kv(h, 0)

            @pl.when(h == HKV - 1)
            def _():
                @pl.loop(0, 16)
                def _(c):
                    _copy(w1_v, dw1_hbm, (slice(None), _ds(c, 8)), sem_out).start()
                    _copy(wo_v, dwo_hbm, (slice(None), _ds(c, 32)), sem_out).start()
                    _copy(w2_v, dw2_hbm, (slice(None), _ds(c, 16)), sem_out).start()
                    _copy(wo_v, dwo_hbm, (pl.ds(0, 3), _ds(16 + c, 32)), sem_out).start()
                    _copy(wq_v, dwq_hbm, (slice(None), _ds(c, 8), pl.ds(0, 2048)), sem_out).start()

            wait_kv(h, 1)

            q, do = q_s[h].astype(BF16), do_s[h].astype(BF16)
            first = lax.broadcasted_iota(jnp.int32, (ROWS, CHUNK), 0) < REP
            for i in range(n_chunks):
                s, dp = [], []
                for b in range(B):
                    tick()
                    s.append(_dot(q, cache(k_v, b, i), NT))
                s_s[:, _ds(i, CHUNK)] = jnp.where(first, s[0], s[1]) * scale
                for b in range(B):
                    tick()
                    dp.append(_dot(do, cache(v_v, b, i), NT))
                dp_s[:, _ds(i, CHUNK)] = jnp.where(first, dp[0], dp[1])

            tick(2)
            s = s_s[...]
            e = jnp.exp(s - jnp.max(s, axis=1, keepdims=True))
            p = e / jnp.sum(e, axis=1, keepdims=True)
            tick(2)
            dp = dp_s[...]
            dscore = p * (dp - jnp.sum(p * dp, axis=1, keepdims=True)) * scale
            pd_s[h] = jnp.concatenate([p, dscore], axis=0).astype(BF16)

            o = [jnp.zeros((2 * ROWS, DH), F32)] * B
            dq = [jnp.zeros((2 * ROWS, DH), F32)] * B
            for i in range(n_chunks):
                for b in range(B):
                    tick()
                    pd = pd_s[h, :, _ds(i, CHUNK)]
                    o[b] = o[b] + _dot(pd, cache(v_v, b, i), NN)
                    dq[b] = dq[b] + _dot(pd, cache(k_v, b, i), NN)

            tick(2)
            o = from_heads(jnp.where(row_h < REP, o[0][:ROWS], o[1][:ROWS])).astype(BF16)
            dq = from_heads(jnp.where(row_h < REP, dq[0][ROWS:], dq[1][ROWS:])).astype(BF16)
            attn_out = attn_out + _dot(o, wo_v[wo_rows(h)], NN)
            tick(2)
            dx = dx + _dot(dq, wq_v[wq_cols(h)].reshape(D, GW), NT)
            tick(4)
            wo_v[wo_rows(h)] = _dot(o, da, TN).astype(BF16)
            tick(4)
            wq_v[wq_cols(h)] = _dot(xb, dq, TN).astype(BF16).reshape(4, D // 4, GW)
            assert issued[0] == ROUNDS
            return attn_out, dx

        attn_out, dx = lax.fori_loop(0, HKV, head, (jnp.zeros((ROWS, D), F32), dx))

        attn_out = per_batch(attn_out)
        out = g * attn_out + (1.0 - g) * ffn_out
        dz = jnp.sum(go8 * (attn_out - ffn_out), axis=1, keepdims=True) * g * (1.0 - g)
        dx = per_batch(dx) + dz * gw
        batch0 = lax.broadcasted_iota(jnp.int32, (B, D), 0) == 0
        out_v[...] = jnp.where(batch0, out[0:1], out[REP:REP + 1]).astype(BF16)
        dx_v[...] = jnp.where(batch0, dx[0:1], dx[REP:REP + 1]).astype(BF16)
        dgw = dz * x8
        dgw = dgw[0:1] + dgw[REP:REP + 1]
        dgw_v[...] = jnp.concatenate(
            [dgw[:, i * LANES:(i + 1) * LANES] for i in range(D // LANES)], axis=0).astype(BF16)

    pl.run_scoped(read_phase, pltpu.SemaphoreType.DMA((3,)), pltpu.SemaphoreType.DMA((2 * HKV,)))

    small_out = [pltpu.make_async_copy(src, dst, sem_out)
                 for src, dst in ((out_v, out_hbm), (dx_v, dx_hbm), (dgw_v, dgw_hbm))]
    for cp in small_out:
        cp.start()

    heads_per_group = GROUP // NSEG
    steps = SEG // WC

    @pl.loop(0, HKV // heads_per_group * steps)
    def _(t):
        grp, i = t // steps, t % steps
        for j in range(heads_per_group):
            h = grp * heads_per_group + j
            q, do = q_s[h], do_s[h]
            zero = jnp.zeros_like(q)
            w = []
            for b in range(B):
                mine = row_h // REP == b
                w.append(jnp.concatenate([zero, jnp.where(mine, q, 0.0)], axis=0))
                w.append(jnp.concatenate([jnp.where(mine, do, 0.0), zero], axis=0))
            w = jnp.concatenate(w, axis=1).astype(BF16)
            for sg in range(NSEG):
                grads = _dot(pd_s[h, :, _ds(sg * steps + i, WC)], w, TN).astype(BF16)
                for b in range(B):
                    seg = (b * HKV + h) * NSEG + sg
                    k_v[seg, _ds(i, WC), :] = grads[:, 2 * b * DH:(2 * b + 1) * DH]
                    v_v[seg, _ds(i, WC), :] = grads[:, (2 * b + 1) * DH:(2 * b + 2) * DH]

        @pl.when((t == 0) | (t % 2 == 1))
        def _():
            lo = jnp.where(t < 2, i, i - 1)
            for src, dst in ((k_v, dk_hbm), (v_v, dv_hbm)):
                for b in range(B):
                    @pl.loop(lo * (WC // PIECE), (i + 1) * (WC // PIECE))
                    def _(c):
                        part = pl.ds(b * HKV * NSEG + grp * GROUP, GROUP)
                        _copy(src, dst, (part, _ds(c, PIECE)), sem_out).start()

    @pl.loop(0, 32)
    def _(c):
        _copy(wq_v, dwq_hbm, (slice(None), _ds(c // 2, 8), _ds(2 + c % 2, 1024)), sem_out).start()
        _copy(wo_v, dwo_hbm, (3, _ds(32 + c, 16)), sem_out).start()

    for cp in small_out:
        cp.wait()
    for src, dst in ((wq_v, dwq_hbm), (wo_v, dwo_hbm), (w1_v, dw1_hbm), (w2_v, dw2_hbm),
                     (k_v, dk_hbm), (v_v, dv_hbm)):
        pltpu.make_async_copy(src, dst, sem_out).wait()


@jax.jit
def pallas_gated_mix__gqa_block_cached__dense_activation_relu__decode_kernel(
    A_x: jax.Array,
    A_k_cache: jax.Array,
    A_v_cache: jax.Array,
    A_wq: jax.Array,
    A_wo: jax.Array,
    B_x: jax.Array,
    B_w1: jax.Array,
    B_w2: jax.Array,
    gate_w: jax.Array,
    grad_out: jax.Array,
):
    del B_x
    views = (KV_VIEW, KV_VIEW, WQ_VIEW, WO_VIEW, W1_VIEW, W2_VIEW)
    in_hbm = pl.BlockSpec(memory_space=pltpu.HBM)
    out, dx, dk, dv, dwq, dwo, dw1, dw2, dgw = pl.pallas_call(
        _kernel,
        out_shape=tuple(jax.ShapeDtypeStruct(s, BF16) for s in ((B, D), (B, D), *views, GATE_VIEW)),
        in_specs=[in_hbm] * 9,
        out_specs=(in_hbm,) * 9,
        scratch_shapes=[
            *(pltpu.VMEM(s, BF16) for s in (*views, (B, D), (B, D), GATE_VIEW, (B, D), (B, D), GATE_VIEW)),
            pltpu.VMEM((HKV, ROWS, DH), F32),
            pltpu.VMEM((HKV, ROWS, DH), F32),
            pltpu.VMEM((ROWS, SK), F32),
            pltpu.VMEM((ROWS, SK), F32),
            pltpu.VMEM((HKV, 2 * ROWS, SK), BF16),
            pltpu.SemaphoreType.DMA(()),
        ],
        compiler_params=pltpu.CompilerParams(
            vmem_limit_bytes=110 * 1024 * 1024, disable_bounds_checks=True),
        name="gated_mix_gqa_relu_decode",
    )(A_x.reshape(B, D), A_k_cache.reshape(KV_VIEW), A_v_cache.reshape(KV_VIEW),
      A_wq.reshape(WQ_VIEW), A_wo.reshape(WO_VIEW), B_w1.reshape(W1_VIEW), B_w2.reshape(W2_VIEW),
      gate_w.reshape(GATE_VIEW), grad_out.reshape(B, D))
    return (out.reshape(A_x.shape), dx.reshape(A_x.shape),
            dk.reshape(A_k_cache.shape), dv.reshape(A_v_cache.shape),
            dwq.reshape(A_wq.shape), dwo.reshape(A_wo.shape),
            dw1.reshape(B_w1.shape), dw2.reshape(B_w2.shape), dgw.reshape(gate_w.shape))
```
